```python
import os as _os
_os.environ.setdefault('JAX_PLATFORMS', 'cpu')
import jax
import jax.numpy as jnp

def _softmax(x, axis=-1):
    return jax.nn.softmax(x, axis=axis)

def _gelu(x):
    return jax.nn.gelu(x, approximate=True)

def _silu(x):
    return jax.nn.silu(x)

def _sigmoid(x):
    return jax.nn.sigmoid(x)

def _layernorm(x, axis=-1, eps=1e-05):
    m = jnp.mean(x, axis=axis, keepdims=True)
    v = jnp.var(x, axis=axis, keepdims=True)
    return (x - m) / jnp.sqrt(v + eps)

def _scatter_add(tgt, idx, src, axis=0):
    return tgt.at[idx].add(src)

def _segment_sum(src, seg, n):
    return jax.ops.segment_sum(src, seg, n)

class _Rng:

    def __init__(self, key):
        self._k = key

    def _next(self):
        self._k, sub = jax.random.split(self._k)
        return sub

    def normal(self, shape):
        return jax.random.normal(self._next(), shape, dtype=jnp.bfloat16)

    def randint(self, lo, hi, shape):
        return jax.random.randint(self._next(), shape, lo, hi, dtype=jnp.int32)

    def uniform(self, shape, lo=0.0, hi=1.0):
        return jax.random.uniform(self._next(), shape, jnp.bfloat16, lo, hi)

    def permutation(self, n):
        return jax.random.permutation(self._next(), n)
kernel_name = 'adaLN_cond__mha_block_cached__geglu_ffn__prompt'

def setup_inputs():
    _rng = _Rng(jax.random.key(int.from_bytes(__import__("os").urandom(4), "little")))
    _w = lambda a: (lambda t: t.astype(jnp.bfloat16) if jnp.issubdtype(t.dtype, jnp.floating) else t)(jnp.asarray(a))

    def _A_setup():
        B, Sq, D = (1, 2048, 512)
        H, Sk, Dh = (32, 2048, 128)
        return {'x': _w((lambda *s: _rng.normal(s) * 0.05)(B, Sq, D)), 'k_cache': _w((lambda *s: _rng.normal(s) * 3.2)(B, H, Sk, Dh)), 'v_cache': _w((lambda *s: _rng.normal(s) * 0.4)(B, H, Sk, Dh)), 'wq': _w((lambda *s: _rng.normal(s) * 1.6)(D, H * Dh) * D ** (-0.5)), 'wo': _w((lambda *s: _rng.normal(s) * 0.4)(H * Dh, D) * (H * Dh) ** (-0.5))}
    _A_in = _A_setup()

    def _B_setup():
        B, S, D, F = (1, 2048, 512, 1792)
        return {'x': _w((lambda *s: _rng.normal(s) * 0.05)(B, S, D)), 'w_gate': _w((lambda *s: _rng.normal(s) * 0.05)(D, F)), 'w_up': _w((lambda *s: _rng.normal(s) * 0.05)(D, F)), 'w_down': _w((lambda *s: _rng.normal(s) * 0.05)(F, D))}
    _B_in = _B_setup()
    return {'A_x': _A_in['x'], 'A_k_cache': _A_in['k_cache'], 'A_v_cache': _A_in['v_cache'], 'A_wq': _A_in['wq'], 'A_wo': _A_in['wo'], 'B_x': _B_in['x'], 'B_w_gate': _B_in['w_gate'], 'B_w_up': _B_in['w_up'], 'B_w_down': _B_in['w_down'], 'c': _w((lambda *s: _rng.normal(s) * 0.05)(1, 512) * 8.0), 'w_mod': _w((lambda *s: _rng.normal(s) * 0.05)(512, 6 * 512) * 512 ** (-0.5) * 8.0)}

def reference(A_x, A_k_cache, A_v_cache, A_wq, A_wo, B_x, B_w_gate, B_w_up, B_w_down, c, w_mod):

    def _A_ref(x, k_cache, v_cache, wq, wo):
        B, Sq, D = x.shape
        H, Dh = (32, 128)
        q = (lambda x, *d: x.transpose(*d))((x @ wq).reshape(B, Sq, H, Dh), 0, 2, 1, 3)
        scores = jnp.einsum('bhqd,bhkd->bhqk', q, k_cache) * Dh ** (-0.5)
        p = _softmax(scores, axis=-1)
        o = jnp.einsum('bhqk,bhkd->bhqd', p, v_cache)
        return (lambda x, *d: x.transpose(*d))(o, 0, 2, 1, 3).reshape(B, Sq, H * Dh) @ wo

    def _B_ref(x, w_gate, w_up, w_down):
        return _gelu(x @ w_gate) * (x @ w_up) @ w_down
    x = A_x
    mod = (_silu(c) @ w_mod).reshape(c.shape[0], 6, 1, -1)
    sa, ca, ga, sb, cb, gb = (mod[:, 0].copy(), mod[:, 1].copy(), mod[:, 2].copy(), mod[:, 3].copy(), mod[:, 4].copy(), mod[:, 5].copy())
    h = _layernorm(x, axis=-1) * (1 + ca) + sa
    x = x + ga * _A_ref(h, A_k_cache, A_v_cache, A_wq, A_wo)
    h = _layernorm(x, axis=-1) * (1 + cb) + sb
    x = x + gb * _B_ref(h, B_w_gate, B_w_up, B_w_down)
    return x
```

```python
import numpy as np
import jax
import jax.numpy as jnp
import jax.experimental.pallas as pl
import jax.experimental.pallas.tpu as pltpu

_O = {}
H, DH, SQ, SK, D, F = 32, 128, 2048, 2048, 512, 1792
BQ = _O.get("BQ", 256)
NB = SQ // BQ
NG = _O.get("NG", 4)
GW = SK // NG
BF = _O.get("BF", 256)
NF = SQ // BF
LB = _O.get("LB", 128)
XC = _O.get("XC", 4)
NSLOT = 4
NHEAD = _O.get("NHEAD", H)
QSC = float(DH ** -0.5 * np.log2(np.e))
SCHED = _O.get("SCHED", "k0 o k1 v0 k2 v1 k3 v2 v3 q")
F32, BF16, U32 = jnp.float32, jnp.bfloat16, jnp.uint32


def _ln_mod(x, scale, shift):
    m = jnp.mean(x, axis=-1, keepdims=True)
    xc = x - m
    v = jnp.mean(xc * xc, axis=-1, keepdims=True)
    return xc * jax.lax.rsqrt(v + 1e-5) * (1.0 + scale) + shift


def _packed(ref, *idx):
    return pltpu.bitcast(ref.bitcast(U32)[idx], BF16)


def kernel(x_hbm, k_hbm, v_hbm, wq_hbm, wo_hbm, wg_hbm, wu_hbm, wd_hbm, c_hbm, wm_hbm,
           o_hbm,
           x_v, k_v, v_v, wq_v, wo_v, wg_v, wu_v, wd_v, c_v, wm_v, o_v,
           mod_v, h_v, acc_v, q_v, p_v, h2_v, x1_v,
           sem_head, sem_misc, sem_x, sem_out):

    def k_copies(h, slot):
        hc = pl.ds(pl.multiple_of(h * DH, DH), DH)
        return [
            pltpu.make_async_copy(wq_hbm.at[:, hc], wq_v.at[slot], sem_head.at[slot, 0]),
            pltpu.make_async_copy(k_hbm.at[h], k_v.at[slot], sem_head.at[slot, 1]),
        ]

    def v_copies(h, slot):
        hc = pl.ds(pl.multiple_of(h * DH, DH), DH)
        return [
            pltpu.make_async_copy(v_hbm.at[h], v_v.at[slot], sem_head.at[slot, 2]),
            pltpu.make_async_copy(wo_hbm.at[hc, :], wo_v.at[slot], sem_head.at[slot, 3]),
        ]

    def head_copies(h, slot):
        return k_copies(h, slot) + v_copies(h, slot)

    XR = SQ // XC
    cp_c = pltpu.make_async_copy(c_hbm, c_v, sem_misc.at[0])
    cp_wma = pltpu.make_async_copy(wm_hbm.at[:, pl.ds(0, 2 * D)], wm_v.at[:, pl.ds(0, 2 * D)], sem_misc.at[1])
    cp_wmb = pltpu.make_async_copy(wm_hbm.at[:, pl.ds(2 * D, 4 * D)], wm_v.at[:, pl.ds(2 * D, 4 * D)], sem_misc.at[2])
    cp_x = [pltpu.make_async_copy(x_hbm.at[pl.ds(j * XR, XR)], x_v.at[pl.ds(j * XR, XR)], sem_x.at[j])
            for j in range(XC)]
    cp_wg = pltpu.make_async_copy(wg_hbm, wg_v, sem_misc.at[3])
    cp_wu = pltpu.make_async_copy(wu_hbm, wu_v, sem_misc.at[4])
    cp_wd = pltpu.make_async_copy(wd_hbm, wd_v, sem_misc.at[5])

    import contextlib
    scope = (lambda n: jax.named_scope(n)) if _O.get("PROF", 0) else (lambda n: contextlib.nullcontext())
    PRO = _O.get("PRO", 1)
    cp_c.start()
    cp_wma.start()
    if PRO == 0:
        for cp in cp_x:
            cp.start()
        for cp in head_copies(0, 0):
            cp.start()
    elif PRO == 1:
        cp_x[0].start()
    elif PRO == 2:
        cp_x[0].start()
        for cp in k_copies(0, 0):
            cp.start()
    elif PRO == 3:
        pass

    with scope("wait_c"):
        cp_c.wait()
    c = c_v[...].astype(F32)
    sc = jnp.broadcast_to((c * jax.nn.sigmoid(c)).astype(BF16), (8, D))
    with scope("wait_wma"):
        cp_wma.wait()
    if PRO == 1:
        for cp in cp_x[1:]:
            cp.start()
        for cp in head_copies(0, 0):
            cp.start()
    elif PRO == 2:
        for cp in cp_x[1:]:
            cp.start()
        for cp in v_copies(0, 0):
            cp.start()
    elif PRO == 3:
        for cp in cp_x:
            cp.start()
        for cp in head_copies(0, 0):
            cp.start()
    with scope("mod_a"):
        mod_a = jnp.dot(sc, wm_v[:, 0:2 * D], preferred_element_type=F32)
        mod_v[:, 0:2 * D] = mod_a
    sa = mod_v[0:1, 0:D]
    ca = mod_v[0:1, D:2 * D]

    for j in range(XC):
        with scope(f"wait_x{j}"):
            cp_x[j].wait()
        if j == _O.get("H1AT", 1):
            for cp in head_copies(1, 1):
                cp.start()

        def ln_body(i, _, j=j):
            r = pl.ds(pl.multiple_of(j * XR + i * LB, LB), LB)
            h_v[r, :] = _ln_mod(x_v[r, :].astype(F32), ca, sa).astype(BF16)
            acc_v[r, :] = jnp.zeros((LB, D), F32)
            return 0
        with scope(f"ln{j}"):
            jax.lax.fori_loop(0, XR // LB, ln_body, 0)

    for cp in head_copies(2, 2):
        cp.start()
    cp_wmb.start()
    cp_wg.start(); cp_wu.start(); cp_wd.start()

    def rows(i):
        return pl.ds(i * BQ if isinstance(i, int) else pl.multiple_of(i * BQ, BQ), BQ)

    def qproj(i, slot):
        q = jnp.dot(h_v[rows(i), :], _packed(wq_v, slot), preferred_element_type=F32)
        return (q * QSC).astype(BF16)

    def qk_soft(q, slot, g, st):
        kk = _packed(k_v, slot, pl.ds(g * GW // 2, GW // 2), slice(None))
        s = jax.lax.dot_general(q, kk, (((1,), (1,)), ((), ())), preferred_element_type=F32)
        if _O.get("MAXM", 0) == 0:
            mg = jnp.max(s, axis=-1, keepdims=True)
        else:
            mm = jnp.maximum(jnp.maximum(s[:, 0:128], s[:, 128:256]), jnp.maximum(s[:, 256:384], s[:, 384:512]))
            mg = jnp.max(mm, axis=-1, keepdims=True)
        if g == 0:
            m_new, alpha = mg, None
        else:
            m_new = jnp.maximum(st["m"], mg)
            alpha = jnp.exp2(st["m"] - m_new)
        p = jnp.exp2(s - m_new)
        if _O.get("LT", 0) == 0:
            lg = p[:, 0:128]
            for j in range(1, GW // 128):
                lg = lg + p[:, j * 128:(j + 1) * 128]
        else:
            lg = (p[:, 0:128] + p[:, 128:256]) + (p[:, 256:384] + p[:, 384:512])
        st["l"] = lg if g == 0 else st["l"] * alpha + lg
        st["m"] = m_new
        if _O.get("PS", 3) == 3:
            p_v[g][pl.ds(pl.multiple_of(st["z"], BQ // 2), BQ // 2), :] = pltpu.bitcast(p.astype(BF16), U32)
        elif _O.get("PS", 3):
            p_v[g][...] = pltpu.bitcast(p.astype(BF16), U32)
        else:
            st["p"][g] = p.astype(BF16)
        st["alpha"][g] = alpha

    def pv(slot, g, st):
        vv = _packed(v_v, slot, pl.ds(g * GW // 2, GW // 2), slice(None))
        if _O.get("PS", 3) == 2:
            pp = pltpu.bitcast(p_v[g][pl.ds(pl.multiple_of(st["z"], BQ // 2), BQ // 2), :], BF16)
        elif _O.get("PS", 3) == 3:
            pp = pltpu.bitcast(p_v[g][...], BF16)
        elif _O.get("PS", 3) == 1:
            pp = pltpu.bitcast(p_v[g][...], BF16)
        else:
            pp = st["p"].pop(g)
        og = jnp.dot(pp, vv, preferred_element_type=F32)
        st["o"] = og if g == 0 else st["o"] * st["alpha"].pop(g) + og

    def finish_o(st):
        l = jnp.sum(st["l"], axis=-1, keepdims=True)
        if _O.get("RCP", 1) == 1:
            return (st["o"] * (1.0 / l)).astype(BF16)
        if _O.get("RCP", 1) == 2:
            return (st["o"] * pl.reciprocal(l)).astype(BF16)
        return (st["o"] / l).astype(BF16)

    def oproj(i, slot, o):
        acc_v[rows(i), :] += jnp.dot(o, _packed(wo_v, slot), preferred_element_type=F32)

    with scope("wait_h0"):
        for cp in head_copies(0, 0):
            cp.wait()
    q_v[...] = pltpu.bitcast(qproj(0, 0), U32)

    UB = _O.get("UB", NB)
    IPH = NB // UB

    def head_body(it, carry):
        h = it // IPH if IPH > 1 else it
        j0 = (it % IPH) * UB if IPH > 1 else 0
        slot = h & (NSLOT - 1)
        nslot = (h + 1) & (NSLOT - 1)

        def waits():
            for cp in head_copies(jnp.minimum(h + 1, H - 1), nslot):
                cp.wait()

        def starts():
            for cp in head_copies(jnp.minimum(h + 3, H - 1), (h + 3) & (NSLOT - 1)):
                cp.start()
        if IPH > 1:
            pl.when(it % IPH == 0)(waits)
        else:
            waits()
        last = (it % IPH == IPH - 1)
        q = pltpu.bitcast(q_v[...], BF16)
        pend = None
        for u in range(UB):
            st = dict(p={}, alpha={}, z=jax.lax.shift_right_logical(it, 16))
            qn = None
            for tok in SCHED.split():
                if tok[0] == "k":
                    qk_soft(q, slot, int(tok[1]), st)
                elif tok[0] == "v":
                    pv(slot, int(tok[1]), st)
                elif tok == "o":
                    if pend is not None:
                        oproj(*pend)
                        pend = None
                elif tok == "q":
                    if u + 1 < UB:
                        qn = qproj(j0 + u + 1, slot)
                    elif IPH == 1:
                        qn = qproj(0, nslot)
                    else:
                        qn = qproj(jnp.where(last, 0, j0 + UB), jnp.where(last, nslot, slot))
            pend = (j0 + u, slot, finish_o(st))
            q = qn
        oproj(*pend)
        q_v[...] = pltpu.bitcast(q, U32)
        if IPH > 1:
            pl.when(last)(starts)
        else:
            starts()
        return carry
    with scope("attn"):
        jax.lax.fori_loop(0, NHEAD * IPH, head_body, 0)
    for j in (NHEAD + 1, NHEAD + 2):
        for cp in head_copies(min(j, H - 1), j % NSLOT):
            cp.wait()

    cp_wmb.wait()
    mod_b = jnp.dot(sc, wm_v[:, 2 * D:6 * D], preferred_element_type=F32)
    ga = mod_b[0:1, 0:D]
    sb = mod_b[0:1, D:2 * D]
    cb = mod_b[0:1, 2 * D:3 * D]
    gb = mod_b[0:1, 3 * D:4 * D]
    cp_wg.wait(); cp_wu.wait(); cp_wd.wait()

    def out_copy(i):
        r = pl.ds(pl.multiple_of(i * BF, BF), BF)
        return pltpu.make_async_copy(o_v.at[r, :], o_hbm.at[r, :], sem_out.at[i])

    def frows(i):
        return pl.ds(i * BF if isinstance(i, int) else pl.multiple_of(i * BF, BF), BF)

    def frows2(i):
        return pl.ds(i * (BF // 2) if isinstance(i, int) else pl.multiple_of(i * (BF // 2), BF // 2), BF // 2)

    def norm2(i):
        r = frows(i)
        x1 = x_v[r, :].astype(F32) + ga * acc_v[r, :]
        x1_v[r, :] = x1
        h2_v[frows2(i), :] = pltpu.bitcast(_ln_mod(x1, cb, sb).astype(BF16), U32)

    def wts(ref):
        return _packed(ref, slice(None), slice(None)) if _O.get("FP", 0) else ref[...]

    NFF = _O.get("NFF", NF)

    def ffn_body(i, _):
        r = frows(i)
        h2 = pltpu.bitcast(h2_v[frows2(i), :], BF16)
        g = jnp.dot(h2, wts(wg_v), preferred_element_type=F32)
        u = jnp.dot(h2, wts(wu_v), preferred_element_type=F32)
        a = (jax.nn.gelu(g, approximate=True) * u).astype(BF16)
        if _O.get("N2POS", 1) == 1:
            norm2(jnp.minimum(i + 1, NF - 1))
        y = jnp.dot(a, wts(wd_v), preferred_element_type=F32)
        if _O.get("N2POS", 1) == 2:
            norm2(jnp.minimum(i + 1, NF - 1))
        o_v[r, :] = (x1_v[r, :] + gb * y).astype(o_v.dtype)
        out_copy(i).start()
        return 0
    norm2(0)
    with scope("ffn"):
        jax.lax.fori_loop(0, NFF, ffn_body, 0)

    def wait_body(i, _):
        out_copy(i).wait()
        return 0
    with scope("wait_out"):
        jax.lax.fori_loop(0, _O.get("NFF", NF), wait_body, 0)


@jax.jit
def pallas_adaLN_cond__mha_block_cached__geglu_ffn__prompt_kernel(A_x, A_k_cache, A_v_cache, A_wq, A_wo, B_x, B_w_gate, B_w_up, B_w_down, c, w_mod):
    del B_x
    x = A_x.reshape(SQ, D)
    k = A_k_cache.reshape(H, SK, DH)
    v = A_v_cache.reshape(H, SK, DH)
    any_spec = pl.BlockSpec(memory_space=pl.ANY)
    out = pl.pallas_call(
        kernel,
        in_specs=[any_spec] * 10,
        out_specs=any_spec,
        out_shape=jax.ShapeDtypeStruct((SQ, D), A_x.dtype),
        scratch_shapes=[
            pltpu.VMEM((SQ, D), BF16),
            pltpu.VMEM((NSLOT, SK, DH), BF16),
            pltpu.VMEM((NSLOT, SK, DH), BF16),
            pltpu.VMEM((NSLOT, D, DH), BF16),
            pltpu.VMEM((NSLOT, DH, D), BF16),
            pltpu.VMEM((D, F), BF16),
            pltpu.VMEM((D, F), BF16),
            pltpu.VMEM((F, D), BF16),
            pltpu.VMEM((1, D), BF16),
            pltpu.VMEM((D, 6 * D), BF16),
            pltpu.VMEM((SQ, D), BF16),
            pltpu.VMEM((8, 6 * D), F32),
            pltpu.VMEM((SQ, D), BF16),
            pltpu.VMEM((SQ, D), F32),
            pltpu.VMEM((BQ // 2, DH), U32),
            [pltpu.VMEM((BQ // 2, GW), U32)] * NG,
            pltpu.VMEM((SQ // 2, D), U32),
            pltpu.VMEM((SQ, D), F32),
            pltpu.SemaphoreType.DMA((NSLOT, 4)),
            pltpu.SemaphoreType.DMA((6,)),
            pltpu.SemaphoreType.DMA((XC,)),
            pltpu.SemaphoreType.DMA((NF,)),
        ],
        compiler_params=pltpu.CompilerParams(
            vmem_limit_bytes=100 * 1024 * 1024,
            disable_bounds_checks=bool(_O.get("NOBC", 1)),
        ),
    )(x, k, v, A_wq, A_wo, B_w_gate, B_w_up, B_w_down, c, w_mod)
    return out.reshape(A_x.shape)
```

```python
import numpy as np
import jax
import jax.numpy as jnp
import jax.experimental.pallas as pl
import jax.experimental.pallas.tpu as pltpu

H, DH, SQ, SK, D, F = 32, 128, 2048, 2048, 512, 1792
NG = 4
GW = SK // NG
BF = 512
NF = SQ // BF
FC = 896
NJ = F // FC
NSLOT = 4
XC = 8
XR = SQ // XC
NC = D // 128
PAD = 8
QSC = float(DH ** -0.5 * np.log2(np.e))
F32, BF16, U32 = jnp.float32, jnp.bfloat16, jnp.uint32


def _packed(ref, *idx):
    return pltpu.bitcast(ref.bitcast(U32)[idx], BF16)


def _cols(v):
    return [v[:, c * 128:(c + 1) * 128] for c in range(v.shape[-1] // 128)]


def _adaln(xs, scale, shift, pins=None, never=None):
    m = jnp.sum((xs[0] + xs[1]) + (xs[2] + xs[3]), axis=-1, keepdims=True) * (1.0 / D)
    if pins is not None:
        m = jnp.where(never, pins[0], m)
    xc = [x - m for x in xs]
    v = jnp.sum((xc[0] * xc[0] + xc[1] * xc[1]) + (xc[2] * xc[2] + xc[3] * xc[3]),
                axis=-1, keepdims=True) * (1.0 / D)
    rs = jax.lax.rsqrt(v + 1e-5)
    if pins is not None:
        rs = jnp.where(never, pins[1], rs)
    return [a * rs * (1.0 + s) + t for a, s, t in zip(xc, _cols(scale), _cols(shift))]


def _kernel(x_hbm, k_hbm, v_hbm, wq_hbm, wo_hbm, wg_hbm, wu_hbm, wd_hbm, c_hbm, wm_hbm,
            o_hbm,
            x_v, k_v, v_v, wq_v, wo_v, wg_v, wu_v, wd_v, c_v, wm_v, o_v,
            mod_v, h_v, acc_v, h2_v, x1_v, fc_v, q_v, p_v, l_v, a_v, oa_v,
            sem_head, sem_misc, sem_x, sem_out):

    def slot_of(h):
        return h % NSLOT if isinstance(h, int) else h & (NSLOT - 1)

    def head_copies(h):
        g = min(h, H - 1) if isinstance(h, int) else jnp.minimum(h, H - 1)
        hc = pl.ds(pl.multiple_of(g * DH, DH), DH)
        s = slot_of(h)
        return (lambda: pltpu.make_async_copy(wq_hbm.at[:, hc], wq_v.at[s], sem_head.at[s, 0]),
                lambda: pltpu.make_async_copy(k_hbm.at[g], k_v.at[s], sem_head.at[s, 1]),
                lambda: pltpu.make_async_copy(v_hbm.at[g], v_v.at[s], sem_head.at[s, 2]),
                lambda: pltpu.make_async_copy(wo_hbm.at[hc, :], wo_v.at[s], sem_head.at[s, 3]))

    def start(h, which=(0, 1, 2, 3)):
        cps = head_copies(h)
        for i in which:
            cps[i]().start()

    def wait(h, which=(0, 1, 2, 3)):
        cps = head_copies(h)
        for i in which:
            cps[i]().wait()

    cp_c = pltpu.make_async_copy(c_hbm, c_v, sem_misc.at[0])
    cp_wma = pltpu.make_async_copy(wm_hbm.at[:, pl.ds(0, 2 * D)], wm_v.at[:, pl.ds(0, 2 * D)], sem_misc.at[1])
    cp_wmb = pltpu.make_async_copy(wm_hbm.at[:, pl.ds(2 * D, 4 * D)], wm_v.at[:, pl.ds(2 * D, 4 * D)], sem_misc.at[2])
    cp_ffn = [pltpu.make_async_copy(wg_hbm, wg_v, sem_misc.at[3]),
              pltpu.make_async_copy(wu_hbm, wu_v, sem_misc.at[4]),
              pltpu.make_async_copy(wd_hbm, wd_v, sem_misc.at[5])]
    cp_x = [pltpu.make_async_copy(x_hbm.at[pl.ds(j * XR, XR)], x_v.at[pl.ds(j * XR, XR)], sem_x.at[j])
            for j in range(XC)]

    cp_c.start()
    cp_wma.start()
    cp_x[0].start()

    cp_c.wait()
    c = c_v[...].astype(F32)
    sc = jnp.broadcast_to((c * jax.nn.sigmoid(c)).astype(BF16), (8, D))
    cp_wma.wait()
    cp_x[1].start()
    mod_v[:, 0:2 * D] = jnp.dot(sc, wm_v[:, 0:2 * D], preferred_element_type=F32)

    def mod_row(k):
        return mod_v[0:1, k * D:(k + 1) * D]

    sa, ca = mod_row(0), mod_row(1)

    def ln1(j):
        r = pl.ds(j * XR, XR)
        xs = [x_v[r, pl.ds(c_ * 128, 128)].astype(F32) for c_ in range(NC)]
        for c_, hh in enumerate(_adaln(xs, ca, sa)):
            h_v[pl.ds(j * XR // 2, XR // 2), pl.ds(c_ * 128, 128)] = pltpu.bitcast(hh.astype(BF16), U32)
        acc_v[r, :] = jnp.zeros((XR, D), F32)

    def qproj(slot):
        h = pltpu.bitcast(h_v[...], BF16)
        q = jnp.dot(h, _packed(wq_v, slot), preferred_element_type=F32)
        q_v[...] = pltpu.bitcast((q * QSC).astype(BF16), U32)

    cp_x[0].wait()
    cp_x[2].start()
    ln1(0)
    cp_x[1].wait()
    cp_x[3].start()
    start(0, (0,))
    ln1(1)
    cp_x[2].wait()
    cp_x[4].start()
    cp_x[5].start()
    ln1(2)
    cp_x[3].wait()
    cp_x[6].start()
    cp_x[7].start()
    start(0, (1,))
    ln1(3)
    for j in range(4, XC):
        cp_x[j].wait()
    wait(0, (0,))
    start(0, (2, 3))
    for j in range(4, XC):
        ln1(j)
    qproj(0)
    start(1)
    start(2)

    def fence(ref, n, z):
        if z is not None:
            ref[pl.ds(pl.multiple_of(n + z, 8), 8), pl.ds(0, 128)] = jnp.zeros((8, 128), ref.dtype)

    def head(slot, z, q_next, post=None):
        q = pltpu.bitcast(q_v[...], BF16)
        st = {}

        def qk(g):
            kk = _packed(k_v, slot, pl.ds(g * GW // 2, GW // 2), slice(None))
            s = jax.lax.dot_general(q, kk, (((1,), (1,)), ((), ())), preferred_element_type=F32)
            mg = jnp.max(s, axis=-1, keepdims=True)
            if g == 0:
                m_new = mg
            else:
                m_new = jnp.maximum(st["m"], mg)
                alpha = jnp.exp2(st["m"] - m_new)
            p = jnp.exp2(s - m_new)
            lg = p[:, 0:128]
            for j in range(1, GW // 128):
                lg = lg + p[:, j * 128:(j + 1) * 128]
            if g > 0:
                lg = l_v[(g - 1) % 2][pl.ds(0, SQ), :] * alpha + lg
                a_v[g % 2][pl.ds(0, SQ), :] = jnp.broadcast_to(alpha, (SQ, DH))
                fence(a_v[g % 2], SQ, z)
            l_v[g % 2][pl.ds(0, SQ), :] = lg
            fence(l_v[g % 2], SQ, z)
            st["m"] = m_new
            p_v[g][pl.ds(0, SQ // 2), :] = pltpu.bitcast(p.astype(BF16), U32)
            fence(p_v[g], SQ // 2, z)

        def pv(g):
            vv = _packed(v_v, slot, pl.ds(g * GW // 2, GW // 2), slice(None))
            og = jnp.dot(pltpu.bitcast(p_v[g][pl.ds(0, SQ // 2), :], BF16), vv, preferred_element_type=F32)
            if g > 0:
                og = oa_v[(g - 1) % 2][pl.ds(0, SQ), :] * a_v[g % 2][pl.ds(0, SQ), :] + og
            if g + 1 < NG:
                oa_v[g % 2][pl.ds(0, SQ), :] = og
                fence(oa_v[g % 2], SQ, z)
            else:
                st["o"] = og

        qk(0); qk(1); pv(0); qk(2); pv(1); qk(3); pv(2)
        q_next()
        pv(3)
        l = jnp.sum(l_v[(NG - 1) % 2][pl.ds(0, SQ), :], axis=-1, keepdims=True)
        o = (st["o"] * (1.0 / l)).astype(BF16)
        new = acc_v[...] + jnp.dot(o, _packed(wo_v, slot), preferred_element_type=F32)
        acc_v[...] = new
        if post is not None:
            post(new)

    def head_body(h, carry):
        wait(h, (1, 2, 3))
        wait(h + 1, (0,))

        @pl.when(h == 1)
        def _():
            cp_wmb.start()
            for cp in cp_ffn:
                cp.start()

        head(slot_of(h), jax.lax.shift_right_logical(h, 16), lambda: qproj(slot_of(h + 1)))
        start(h + 3)
        return carry
    jax.lax.fori_loop(0, H - 1, head_body, 0)

    def norm2(r0, attn=None, pins=None, never=None):
        r = pl.ds(r0, BF)
        r2 = pl.ds(r0 // 2 if isinstance(r0, int) else pl.multiple_of(r0 // 2, BF // 2), BF // 2)
        at = [acc_v[r, pl.ds(c_ * 128, 128)] for c_ in range(NC)] if attn is None else _cols(attn)
        xs = [x_v[r, pl.ds(c_ * 128, 128)].astype(F32) + g_ * a_
              for c_, (g_, a_) in enumerate(zip(_cols(mod_row(2)), at))]
        for c_, hh in enumerate(_adaln(xs, mod_row(4), mod_row(3), pins, never)):
            x1_v[r, pl.ds(c_ * 128, 128)] = xs[c_]
            h2_v[r2, pl.ds(c_ * 128, 128)] = pltpu.bitcast(hh.astype(BF16), U32)

    def mod_b():
        mod_v[:, 2 * D:6 * D] = jnp.dot(sc, wm_v[:, 2 * D:6 * D], preferred_element_type=F32)

    wait(H - 1, (1, 2, 3))
    cp_wmb.wait()
    head(slot_of(H - 1), None, mod_b, lambda new: norm2(0, new[0:BF]))

    for cp in cp_ffn:
        cp.wait()

    def out_copy(i):
        r = pl.ds(pl.multiple_of(i * BF, BF), BF)
        return pltpu.make_async_copy(o_v.at[r, :], o_hbm.at[r, :], sem_out.at[i])

    def ffn_body(i, carry):
        r = pl.ds(pl.multiple_of(i * BF, BF), BF)
        z = jax.lax.shift_right_logical(i, 16)
        h2 = pltpu.bitcast(h2_v[pl.ds(pl.multiple_of(i * (BF // 2), BF // 2), BF // 2), :], BF16)
        for j in range(NJ):
            g = jnp.dot(h2, wg_v[:, pl.ds(j * FC, FC)], preferred_element_type=F32)
            u = jnp.dot(h2, wu_v[:, pl.ds(j * FC, FC)], preferred_element_type=F32)
            if j == 0:
                nxt = pl.multiple_of(jnp.minimum(i + 1, NF - 1) * BF, BF)
                norm2(nxt, None, [g[:, 0:128], g[:, FC - 128:FC]], z != 0)
            a = (jax.nn.gelu(g, approximate=True) * u).astype(BF16)
            fc_v[j][pl.ds(pl.multiple_of(z, BF // 2), BF // 2), :] = pltpu.bitcast(a, U32)
        aa = jnp.concatenate([pltpu.bitcast(fc_v[j][pl.ds(0, BF // 2), :], BF16) for j in range(NJ)], axis=1)
        y = jnp.dot(aa, wd_v[...], preferred_element_type=F32)
        o_v[r, :] = (x1_v[r, :] + mod_row(5) * y).astype(o_v.dtype)
        out_copy(i).start()
        return carry
    jax.lax.fori_loop(0, NF, ffn_body, 0)

    wait(H)
    wait(H + 1)

    def wait_body(i, carry):
        out_copy(i).wait()
        return carry
    jax.lax.fori_loop(0, NF, wait_body, 0)


@jax.jit
def pallas_adaLN_cond__mha_block_cached__geglu_ffn__prompt_kernel(
    A_x: jax.Array,
    A_k_cache: jax.Array,
    A_v_cache: jax.Array,
    A_wq: jax.Array,
    A_wo: jax.Array,
    B_x: jax.Array,
    B_w_gate: jax.Array,
    B_w_up: jax.Array,
    B_w_down: jax.Array,
    c: jax.Array,
    w_mod: jax.Array,
):
    del B_x
    x = A_x.reshape(SQ, D)
    k = A_k_cache.reshape(H, SK, DH)
    v = A_v_cache.reshape(H, SK, DH)
    any_spec = pl.BlockSpec(memory_space=pl.ANY)
    out = pl.pallas_call(
        _kernel,
        in_specs=[any_spec] * 10,
        out_specs=any_spec,
        out_shape=jax.ShapeDtypeStruct((SQ, D), A_x.dtype),
        scratch_shapes=[
            pltpu.VMEM((SQ, D), BF16),
            pltpu.VMEM((NSLOT, SK, DH), BF16),
            pltpu.VMEM((NSLOT, SK, DH), BF16),
            pltpu.VMEM((NSLOT, D, DH), BF16),
            pltpu.VMEM((NSLOT, DH, D), BF16),
            pltpu.VMEM((D, F), BF16),
            pltpu.VMEM((D, F), BF16),
            pltpu.VMEM((F, D), BF16),
            pltpu.VMEM((1, D), BF16),
            pltpu.VMEM((D, 6 * D), BF16),
            pltpu.VMEM((SQ, D), BF16),
            pltpu.VMEM((8, 6 * D), F32),
            pltpu.VMEM((SQ // 2, D), U32),
            pltpu.VMEM((SQ, D), F32),
            pltpu.VMEM((SQ // 2, D), U32),
            pltpu.VMEM((SQ, D), F32),
            [pltpu.VMEM((BF // 2 + PAD, FC), U32)] * NJ,
            pltpu.VMEM((SQ // 2, DH), U32),
            [pltpu.VMEM((SQ // 2 + PAD, GW), U32)] * NG,
            [pltpu.VMEM((SQ + PAD, DH), F32)] * 2,
            [pltpu.VMEM((SQ + PAD, DH), F32)] * 2,
            [pltpu.VMEM((SQ + PAD, DH), F32)] * 2,
            pltpu.SemaphoreType.DMA((NSLOT, 4)),
            pltpu.SemaphoreType.DMA((6,)),
            pltpu.SemaphoreType.DMA((XC,)),
            pltpu.SemaphoreType.DMA((NF,)),
        ],
        compiler_params=pltpu.CompilerParams(
            vmem_limit_bytes=100 * 1024 * 1024,
            disable_bounds_checks=True,
        ),
    )(x, k, v, A_wq, A_wo, B_w_gate, B_w_up, B_w_down, c, w_mod)
    return out.reshape(A_x.shape)
```

```python
import numpy as np
import jax
import jax.numpy as jnp
import jax.experimental.pallas as pl
import jax.experimental.pallas.tpu as pltpu

H, DH, SQ, SK, D, F = 32, 128, 2048, 2048, 512, 1792
NG = 4
GW = SK // NG
BF = 512
NF = SQ // BF
FC = 896
NJ = F // FC
NSLOT = 4
XC = 8
XR = SQ // XC
NC = D // 128
NO = 4
OR = BF // NO
PAD = 8
QSC = float(DH ** -0.5 * np.log2(np.e))
F32, BF16, U32 = jnp.float32, jnp.bfloat16, jnp.uint32


def _packed(ref, *idx):
    return pltpu.bitcast(ref.bitcast(U32)[idx], BF16)


def _cols(v):
    return [v[:, c * 128:(c + 1) * 128] for c in range(v.shape[-1] // 128)]


def _adaln(xs, scale, shift, pins=None, never=None):
    m = jnp.sum((xs[0] + xs[1]) + (xs[2] + xs[3]), axis=-1, keepdims=True) * (1.0 / D)
    if pins is not None:
        m = jnp.where(never, pins[0], m)
    xc = [x - m for x in xs]
    v = jnp.sum((xc[0] * xc[0] + xc[1] * xc[1]) + (xc[2] * xc[2] + xc[3] * xc[3]),
                axis=-1, keepdims=True) * (1.0 / D)
    rs = jax.lax.rsqrt(v + 1e-5)
    if pins is not None:
        rs = jnp.where(never, pins[1], rs)
    return [a * rs * (1.0 + s) + t for a, s, t in zip(xc, _cols(scale), _cols(shift))]


def _kernel(x_hbm, k_hbm, v_hbm, wq_hbm, wo_hbm, wg_hbm, wu_hbm, wd_hbm, c_hbm, wm_hbm,
            o_hbm,
            x_v, k_v, v_v, wq_v, wo_v, wg_v, wu_v, wd_v, c_v, wm_v, o_v,
            mod_v, h_v, acc_v, h2_v, x1_v, fc_v, p_v, l_v, a_v, oa_v,
            sem_head, sem_misc, sem_x, sem_out):

    def slot_of(h):
        return h % NSLOT if isinstance(h, int) else h & (NSLOT - 1)

    def head_copies(h):
        g = min(h, H - 1) if isinstance(h, int) else jnp.minimum(h, H - 1)
        hc = pl.ds(pl.multiple_of(g * DH, DH), DH)
        s = slot_of(h)
        return (lambda: pltpu.make_async_copy(wq_hbm.at[:, hc], wq_v.at[s], sem_head.at[s, 0]),
                lambda: pltpu.make_async_copy(k_hbm.at[g], k_v.at[s], sem_head.at[s, 1]),
                lambda: pltpu.make_async_copy(v_hbm.at[g], v_v.at[s], sem_head.at[s, 2]),
                lambda: pltpu.make_async_copy(wo_hbm.at[hc, :], wo_v.at[s], sem_head.at[s, 3]))

    def start(h, which=(0, 1, 2, 3)):
        cps = head_copies(h)
        for i in which:
            cps[i]().start()

    def wait(h, which=(0, 1, 2, 3)):
        cps = head_copies(h)
        for i in which:
            cps[i]().wait()

    cp_c = pltpu.make_async_copy(c_hbm, c_v, sem_misc.at[0])
    cp_wma = pltpu.make_async_copy(wm_hbm.at[:, pl.ds(0, 2 * D)], wm_v.at[:, pl.ds(0, 2 * D)], sem_misc.at[1])
    cp_wmb = pltpu.make_async_copy(wm_hbm.at[:, pl.ds(2 * D, 4 * D)], wm_v.at[:, pl.ds(2 * D, 4 * D)], sem_misc.at[2])
    cp_ffn = [pltpu.make_async_copy(wg_hbm, wg_v, sem_misc.at[3]),
              pltpu.make_async_copy(wu_hbm, wu_v, sem_misc.at[4]),
              pltpu.make_async_copy(wd_hbm, wd_v, sem_misc.at[5])]
    cp_x = [pltpu.make_async_copy(x_hbm.at[pl.ds(j * XR, XR)], x_v.at[pl.ds(j * XR, XR)], sem_x.at[j])
            for j in range(XC)]

    cp_c.start()
    cp_wma.start()
    cp_x[0].start()
    acc_v[...] = jnp.zeros((SQ, D), F32)

    cp_c.wait()
    c = c_v[...].astype(F32)
    sc = jnp.broadcast_to((c * jax.nn.sigmoid(c)).astype(BF16), (8, D))
    cp_wma.wait()
    cp_x[1].start()
    mod_v[:, 0:2 * D] = jnp.dot(sc, wm_v[:, 0:2 * D], preferred_element_type=F32)

    def mod_row(k):
        return mod_v[0:1, k * D:(k + 1) * D]

    sa, ca = mod_row(0), mod_row(1)

    def ln1(j):
        r = pl.ds(j * XR, XR)
        xs = [x_v[r, pl.ds(c_ * 128, 128)].astype(F32) for c_ in range(NC)]
        for c_, hh in enumerate(_adaln(xs, ca, sa)):
            h_v[pl.ds(j * XR // 2, XR // 2), pl.ds(c_ * 128, 128)] = pltpu.bitcast(hh.astype(BF16), U32)

    cp_x[0].wait()
    cp_x[2].start()
    start(0, (0,))
    ln1(0)
    cp_x[1].wait()
    cp_x[3].start()
    cp_x[4].start()
    ln1(1)
    cp_x[2].wait()
    for j in range(5, XC):
        cp_x[j].start()
    ln1(2)
    cp_x[3].wait()
    start(0, (1,))
    ln1(3)
    for j in range(4, XC):
        cp_x[j].wait()
    start(0, (2, 3))
    for j in range(4, XC):
        ln1(j)
    start(1)
    start(2)

    def fence(ref, n, z):
        if z is not None:
            ref[pl.ds(pl.multiple_of(n + z, 8), 8), pl.ds(0, 128)] = jnp.zeros((8, 128), ref.dtype)

    def head(slot, z, post=None):
        q = jnp.dot(pltpu.bitcast(h_v[...], BF16), _packed(wq_v, slot), preferred_element_type=F32)
        q = (q * QSC).astype(BF16)
        st = {}

        def qk(g):
            kk = _packed(k_v, slot, pl.ds(g * GW // 2, GW // 2), slice(None))
            s = jax.lax.dot_general(q, kk, (((1,), (1,)), ((), ())), preferred_element_type=F32)
            mg = jnp.max(s, axis=-1, keepdims=True)
            if g == 0:
                m_new = mg
            else:
                m_new = jnp.maximum(st["m"], mg)
                alpha = jnp.exp2(st["m"] - m_new)
            p = jnp.exp2(s - m_new)
            lg = p[:, 0:128]
            for j in range(1, GW // 128):
                lg = lg + p[:, j * 128:(j + 1) * 128]
            if g > 0:
                lg = l_v[(g - 1) % 2][pl.ds(0, SQ), :] * alpha + lg
                a_v[g % 2][pl.ds(0, SQ), :] = jnp.broadcast_to(alpha, (SQ, DH))
                fence(a_v[g % 2], SQ, z)
            l_v[g % 2][pl.ds(0, SQ), :] = lg
            fence(l_v[g % 2], SQ, z)
            st["m"] = m_new
            p_v[g][pl.ds(0, SQ // 2), :] = pltpu.bitcast(p.astype(BF16), U32)
            fence(p_v[g], SQ // 2, z)

        def pv(g):
            vv = _packed(v_v, slot, pl.ds(g * GW // 2, GW // 2), slice(None))
            og = jnp.dot(pltpu.bitcast(p_v[g][pl.ds(0, SQ // 2), :], BF16), vv, preferred_element_type=F32)
            if g > 0:
                og = oa_v[(g - 1) % 2][pl.ds(0, SQ), :] * a_v[g % 2][pl.ds(0, SQ), :] + og
            if g + 1 < NG:
                oa_v[g % 2][pl.ds(0, SQ), :] = og
                fence(oa_v[g % 2], SQ, z)
            else:
                st["o"] = og

        qk(0); qk(1); pv(0); qk(2); pv(1); qk(3); pv(2); pv(3)
        l = jnp.sum(l_v[(NG - 1) % 2][pl.ds(0, SQ), :], axis=-1, keepdims=True)
        o = (st["o"] * (1.0 / l)).astype(BF16)
        new = acc_v[...] + jnp.dot(o, _packed(wo_v, slot), preferred_element_type=F32)
        acc_v[...] = new
        if post is not None:
            post(new)

    def head_body(h, carry):
        wait(h)

        @pl.when(h == 1)
        def _():
            cp_wmb.start()
            for cp in cp_ffn:
                cp.start()

        head(slot_of(h), jax.lax.shift_right_logical(h, 16))
        start(h + 3)
        return carry | jax.lax.shift_right_logical(h, 16)
    z_out = jax.lax.fori_loop(0, H - 1, head_body, jnp.int32(0))

    def norm2(r0, attn, pins, never):
        r = pl.ds(r0, BF)
        r2 = pl.ds(r0 // 2 if isinstance(r0, int) else pl.multiple_of(r0 // 2, BF // 2), BF // 2)
        at = [acc_v[r, pl.ds(c_ * 128, 128)] for c_ in range(NC)] if attn is None else _cols(attn)
        xs = [x_v[r, pl.ds(c_ * 128, 128)].astype(F32) + g_ * a_
              for c_, (g_, a_) in enumerate(zip(_cols(mod_row(2)), at))]
        for c_, hh in enumerate(_adaln(xs, mod_row(4), mod_row(3), pins, never)):
            x1_v[r, pl.ds(c_ * 128, 128)] = xs[c_]
            h2_v[r2, pl.ds(c_ * 128, 128)] = pltpu.bitcast(hh.astype(BF16), U32)

    def first_norm2(attn):
        norm2(0, attn[0:BF], [attn[BF:2 * BF, 0:128], attn[2 * BF:3 * BF, 0:128]], z_out != 0)

    wait(H - 1)
    cp_wmb.wait()
    mod_v[:, 2 * D:6 * D] = jnp.dot(sc, wm_v[:, 2 * D:6 * D], preferred_element_type=F32)
    head(slot_of(H - 1), None, first_norm2)

    for cp in cp_ffn:
        cp.wait()

    def out_rows(i, t):
        return pl.ds(pl.multiple_of(i * BF + t * OR, OR), OR)

    def out_copy(i, t):
        return pltpu.make_async_copy(o_v.at[out_rows(i, t), :], o_hbm.at[out_rows(i, t), :], sem_out.at[i, t])

    def ffn_body(i, carry):
        r = pl.ds(pl.multiple_of(i * BF, BF), BF)
        z = jax.lax.shift_right_logical(i, 16)
        h2 = pltpu.bitcast(h2_v[pl.ds(pl.multiple_of(i * (BF // 2), BF // 2), BF // 2), :], BF16)
        for j in range(NJ):
            g = jnp.dot(h2, wg_v[:, pl.ds(j * FC, FC)], preferred_element_type=F32)
            u = jnp.dot(h2, wu_v[:, pl.ds(j * FC, FC)], preferred_element_type=F32)
            if j == 0:
                nxt = pl.multiple_of(jnp.minimum(i + 1, NF - 1) * BF, BF)
                norm2(nxt, None, [g[:, 0:128], g[:, FC - 128:FC]], z != 0)
            a = (jax.nn.gelu(g, approximate=True) * u).astype(BF16)
            fc_v[j][pl.ds(pl.multiple_of(z, BF // 2), BF // 2), :] = pltpu.bitcast(a, U32)
        aa = jnp.concatenate([pltpu.bitcast(fc_v[j][pl.ds(0, BF // 2), :], BF16) for j in range(NJ)], axis=1)
        y = jnp.dot(aa, wd_v[...], preferred_element_type=F32)
        res = (x1_v[r, :] + mod_row(5) * y).astype(o_v.dtype)
        for t in range(NO):
            o_v[out_rows(i, t), :] = res[t * OR:(t + 1) * OR]
            out_copy(i, t).start()
        return carry
    jax.lax.fori_loop(0, NF, ffn_body, 0)

    wait(H)
    wait(H + 1)

    def wait_body(i, carry):
        for t in range(NO):
            out_copy(i, t).wait()
        return carry
    jax.lax.fori_loop(0, NF, wait_body, 0)


@jax.jit
def pallas_adaLN_cond__mha_block_cached__geglu_ffn__prompt_kernel(
    A_x: jax.Array,
    A_k_cache: jax.Array,
    A_v_cache: jax.Array,
    A_wq: jax.Array,
    A_wo: jax.Array,
    B_x: jax.Array,
    B_w_gate: jax.Array,
    B_w_up: jax.Array,
    B_w_down: jax.Array,
    c: jax.Array,
    w_mod: jax.Array,
):
    del B_x
    x = A_x.reshape(SQ, D)
    k = A_k_cache.reshape(H, SK, DH)
    v = A_v_cache.reshape(H, SK, DH)
    any_spec = pl.BlockSpec(memory_space=pl.ANY)
    out = pl.pallas_call(
        _kernel,
        in_specs=[any_spec] * 10,
        out_specs=any_spec,
        out_shape=jax.ShapeDtypeStruct((SQ, D), A_x.dtype),
        scratch_shapes=[
            pltpu.VMEM((SQ, D), BF16),
            pltpu.VMEM((NSLOT, SK, DH), BF16),
            pltpu.VMEM((NSLOT, SK, DH), BF16),
            pltpu.VMEM((NSLOT, D, DH), BF16),
            pltpu.VMEM((NSLOT, DH, D), BF16),
            pltpu.VMEM((D, F), BF16),
            pltpu.VMEM((D, F), BF16),
            pltpu.VMEM((F, D), BF16),
            pltpu.VMEM((1, D), BF16),
            pltpu.VMEM((D, 6 * D), BF16),
            pltpu.VMEM((SQ, D), BF16),
            pltpu.VMEM((8, 6 * D), F32),
            pltpu.VMEM((SQ // 2, D), U32),
            pltpu.VMEM((SQ, D), F32),
            pltpu.VMEM((SQ // 2, D), U32),
            pltpu.VMEM((SQ, D), F32),
            [pltpu.VMEM((BF // 2 + PAD, FC), U32)] * NJ,
            [pltpu.VMEM((SQ // 2 + PAD, GW), U32)] * NG,
            [pltpu.VMEM((SQ + PAD, DH), F32)] * 2,
            [pltpu.VMEM((SQ + PAD, DH), F32)] * 2,
            [pltpu.VMEM((SQ + PAD, DH), F32)] * 2,
            pltpu.SemaphoreType.DMA((NSLOT, 4)),
            pltpu.SemaphoreType.DMA((6,)),
            pltpu.SemaphoreType.DMA((XC,)),
            pltpu.SemaphoreType.DMA((NF, NO)),
        ],
        compiler_params=pltpu.CompilerParams(
            vmem_limit_bytes=100 * 1024 * 1024,
            disable_bounds_checks=True,
        ),
    )(x, k, v, A_wq, A_wo, B_w_gate, B_w_up, B_w_down, c, w_mod)
    return out.reshape(A_x.shape)
```

```python
import numpy as np
import jax
import jax.numpy as jnp
import jax.experimental.pallas as pl
import jax.experimental.pallas.tpu as pltpu

H, DH, SQ, SK, D, F = 32, 128, 2048, 2048, 512, 1792
NG = 4
GW = SK // NG
BF = 512
NF = SQ // BF
FC = 896
NJ = F // FC
NSLOT = 4
XC = 8
XR = SQ // XC
NC = D // 128
NO = 4
OR = BF // NO
PAD = 8
QSC = float(DH ** -0.5 * np.log2(np.e))
F32, BF16, U32 = jnp.float32, jnp.bfloat16, jnp.uint32


def _packed(ref, *idx):
    return pltpu.bitcast(ref.bitcast(U32)[idx], BF16)


def _cols(v):
    return [v[:, c * 128:(c + 1) * 128] for c in range(v.shape[-1] // 128)]


def _adaln(xs, scale, shift, pins=None, never=None):
    m = jnp.sum((xs[0] + xs[1]) + (xs[2] + xs[3]), axis=-1, keepdims=True) * (1.0 / D)
    if pins is not None:
        m = jnp.where(never, pins[0], m)
    xc = [x - m for x in xs]
    v = jnp.sum((xc[0] * xc[0] + xc[1] * xc[1]) + (xc[2] * xc[2] + xc[3] * xc[3]),
                axis=-1, keepdims=True) * (1.0 / D)
    rs = jax.lax.rsqrt(v + 1e-5)
    if pins is not None:
        rs = jnp.where(never, pins[1], rs)
    return [a * rs * (1.0 + s) + t for a, s, t in zip(xc, _cols(scale), _cols(shift))]


def _kernel(x_hbm, k_hbm, v_hbm, wq_hbm, wo_hbm, wg_hbm, wu_hbm, wd_hbm, c_hbm, wm_hbm,
            o_hbm,
            x_v, k_v, v_v, wq_v, wo_v, wg_v, wu_v, wd_v, c_v, wm_v, o_v,
            mod_v, h_v, acc_v, h2_v, x1_v, fc_v, p_v, l_v, a_v, oa_v,
            sem_head, sem_misc, sem_x, sem_out):

    def slot_of(h):
        return h % NSLOT if isinstance(h, int) else h & (NSLOT - 1)

    def head_copies(h):
        g = min(h, H - 1) if isinstance(h, int) else jnp.minimum(h, H - 1)
        hc = pl.ds(pl.multiple_of(g * DH, DH), DH)
        s = slot_of(h)
        return (pltpu.make_async_copy(wq_hbm.at[:, hc], wq_v.at[s], sem_head.at[s, 0]),
                pltpu.make_async_copy(k_hbm.at[g], k_v.at[s], sem_head.at[s, 1]),
                pltpu.make_async_copy(v_hbm.at[g], v_v.at[s], sem_head.at[s, 2]),
                pltpu.make_async_copy(wo_hbm.at[hc, :], wo_v.at[s], sem_head.at[s, 3]))

    def start(h):
        for cp in head_copies(h):
            cp.start()

    def wait(h):
        for cp in head_copies(h):
            cp.wait()

    cp_c = pltpu.make_async_copy(c_hbm, c_v, sem_misc.at[0])
    cp_wma = pltpu.make_async_copy(wm_hbm.at[:, pl.ds(0, 2 * D)], wm_v.at[:, pl.ds(0, 2 * D)], sem_misc.at[1])
    cp_wmb = pltpu.make_async_copy(wm_hbm.at[:, pl.ds(2 * D, 4 * D)], wm_v.at[:, pl.ds(2 * D, 4 * D)], sem_misc.at[2])
    cp_ffn = [pltpu.make_async_copy(wg_hbm, wg_v, sem_misc.at[3]),
              pltpu.make_async_copy(wu_hbm, wu_v, sem_misc.at[4]),
              pltpu.make_async_copy(wd_hbm, wd_v, sem_misc.at[5])]
    cp_x = [pltpu.make_async_copy(x_hbm.at[pl.ds(j * XR, XR)], x_v.at[pl.ds(j * XR, XR)], sem_x.at[j])
            for j in range(XC)]

    cp_c.start()
    cp_wma.start()
    cp_x[0].start()
    cp_x[1].start()
    acc_v[...] = jnp.zeros((SQ, D), F32)

    cp_c.wait()
    c = c_v[...].astype(F32)
    sc = jnp.broadcast_to((c * jax.nn.sigmoid(c)).astype(BF16), (8, D))
    cp_wma.wait()
    cp_x[2].start()
    cp_x[3].start()
    mod_v[:, 0:2 * D] = jnp.dot(sc, wm_v[:, 0:2 * D], preferred_element_type=F32)

    def mod_row(k):
        return mod_v[0:1, k * D:(k + 1) * D]

    def ln1(j):
        r = pl.ds(j * XR, XR)
        xs = [x_v[r, pl.ds(c_ * 128, 128)].astype(F32) for c_ in range(NC)]
        for c_, hh in enumerate(_adaln(xs, mod_row(1), mod_row(0))):
            h_v[pl.ds(j * XR // 2, XR // 2), pl.ds(c_ * 128, 128)] = pltpu.bitcast(hh.astype(BF16), U32)

    cp_x[0].wait()
    ln1(0)
    cp_x[1].wait()
    for j in range(4, XC):
        cp_x[j].start()
    ln1(1)
    cp_x[2].wait()
    ln1(2)
    cp_x[3].wait()
    start(0)
    ln1(3)
    for j in range(4, XC):
        cp_x[j].wait()
    for j in range(4, XC):
        ln1(j)
    start(1)
    start(2)

    def fence(ref, n, z):
        if z is not None:
            ref[pl.ds(pl.multiple_of(n + z, 8), 8), pl.ds(0, 128)] = jnp.zeros((8, 128), ref.dtype)

    def head(slot, z, post=None):
        q = jnp.dot(pltpu.bitcast(h_v[...], BF16), _packed(wq_v, slot), preferred_element_type=F32)
        q = (q * QSC).astype(BF16)
        st = {}

        def qk(g):
            kk = _packed(k_v, slot, pl.ds(g * GW // 2, GW // 2), slice(None))
            s = jax.lax.dot_general(q, kk, (((1,), (1,)), ((), ())), preferred_element_type=F32)
            mg = jnp.max(s, axis=-1, keepdims=True)
            if g == 0:
                m_new = mg
            else:
                m_new = jnp.maximum(st["m"], mg)
                alpha = jnp.exp2(st["m"] - m_new)
            p = jnp.exp2(s - m_new)
            lg = p[:, 0:128]
            for j in range(1, GW // 128):
                lg = lg + p[:, j * 128:(j + 1) * 128]
            if g > 0:
                lg = l_v[(g - 1) % 2][pl.ds(0, SQ), :] * alpha + lg
                a_v[g % 2][pl.ds(0, SQ), :] = jnp.broadcast_to(alpha, (SQ, DH))
                fence(a_v[g % 2], SQ, z)
            l_v[g % 2][pl.ds(0, SQ), :] = lg
            fence(l_v[g % 2], SQ, z)
            st["m"] = m_new
            p_v[g][pl.ds(0, SQ // 2), :] = pltpu.bitcast(p.astype(BF16), U32)
            fence(p_v[g], SQ // 2, z)

        def pv(g):
            vv = _packed(v_v, slot, pl.ds(g * GW // 2, GW // 2), slice(None))
            og = jnp.dot(pltpu.bitcast(p_v[g][pl.ds(0, SQ // 2), :], BF16), vv, preferred_element_type=F32)
            if g > 0:
                og = oa_v[(g - 1) % 2][pl.ds(0, SQ), :] * a_v[g % 2][pl.ds(0, SQ), :] + og
            if g + 1 < NG:
                oa_v[g % 2][pl.ds(0, SQ), :] = og
                fence(oa_v[g % 2], SQ, z)
            else:
                st["o"] = og

        qk(0); qk(1); pv(0); qk(2); pv(1); qk(3); pv(2); pv(3)
        l = jnp.sum(l_v[(NG - 1) % 2][pl.ds(0, SQ), :], axis=-1, keepdims=True)
        o = (st["o"] * (1.0 / l)).astype(BF16)
        new = acc_v[...] + jnp.dot(o, _packed(wo_v, slot), preferred_element_type=F32)
        acc_v[...] = new
        if post is not None:
            post(new)

    def head_body(h, carry):
        wait(h)

        @pl.when(h == 1)
        def _():
            cp_wmb.start()
            for cp in cp_ffn:
                cp.start()

        head(slot_of(h), jax.lax.shift_right_logical(h, 16))
        start(h + 3)
        return carry | jax.lax.shift_right_logical(h, 16)
    z_out = jax.lax.fori_loop(0, H - 1, head_body, jnp.int32(0))

    def norm2(r0, attn, pins, never):
        r = pl.ds(r0, BF)
        r2 = pl.ds(r0 // 2 if isinstance(r0, int) else pl.multiple_of(r0 // 2, BF // 2), BF // 2)
        at = [acc_v[r, pl.ds(c_ * 128, 128)] for c_ in range(NC)] if attn is None else _cols(attn)
        xs = [x_v[r, pl.ds(c_ * 128, 128)].astype(F32) + g_ * a_
              for c_, (g_, a_) in enumerate(zip(_cols(mod_row(2)), at))]
        for c_, hh in enumerate(_adaln(xs, mod_row(4), mod_row(3), pins, never)):
            x1_v[r, pl.ds(c_ * 128, 128)] = xs[c_]
            h2_v[r2, pl.ds(c_ * 128, 128)] = pltpu.bitcast(hh.astype(BF16), U32)

    def first_norm2(attn):
        norm2(0, attn[0:BF], [attn[BF:2 * BF, 0:128], attn[2 * BF:3 * BF, 0:128]], z_out != 0)

    wait(H - 1)
    cp_wmb.wait()
    mod_v[:, 2 * D:6 * D] = jnp.dot(sc, wm_v[:, 2 * D:6 * D], preferred_element_type=F32)
    head(slot_of(H - 1), None, first_norm2)

    for cp in cp_ffn:
        cp.wait()

    def out_rows(i, t):
        return pl.ds(pl.multiple_of(i * BF + t * OR, OR), OR)

    def out_copy(i, t):
        return pltpu.make_async_copy(o_v.at[out_rows(i, t), :], o_hbm.at[out_rows(i, t), :], sem_out.at[i, t])

    def ffn_body(i, carry):
        r = pl.ds(pl.multiple_of(i * BF, BF), BF)
        z = jax.lax.shift_right_logical(i, 16)
        h2 = pltpu.bitcast(h2_v[pl.ds(pl.multiple_of(i * (BF // 2), BF // 2), BF // 2), :], BF16)
        for j in range(NJ):
            g = jnp.dot(h2, wg_v[:, pl.ds(j * FC, FC)], preferred_element_type=F32)
            u = jnp.dot(h2, wu_v[:, pl.ds(j * FC, FC)], preferred_element_type=F32)
            if j == 0:
                nxt = pl.multiple_of(jnp.minimum(i + 1, NF - 1) * BF, BF)
                norm2(nxt, None, [g[:, 0:128], g[:, FC - 128:FC]], z != 0)
            a = (jax.nn.gelu(g, approximate=True) * u).astype(BF16)
            fc_v[j][pl.ds(pl.multiple_of(z, BF // 2), BF // 2), :] = pltpu.bitcast(a, U32)
        aa = jnp.concatenate([pltpu.bitcast(fc_v[j][pl.ds(0, BF // 2), :], BF16) for j in range(NJ)], axis=1)
        y = jnp.dot(aa, wd_v[...], preferred_element_type=F32)
        res = (x1_v[r, :] + mod_row(5) * y).astype(o_v.dtype)
        for t in range(NO):
            o_v[out_rows(i, t), :] = res[t * OR:(t + 1) * OR]
            out_copy(i, t).start()
        return carry
    jax.lax.fori_loop(0, NF, ffn_body, 0)

    wait(H)
    wait(H + 1)

    def wait_body(i, carry):
        for t in range(NO):
            out_copy(i, t).wait()
        return carry
    jax.lax.fori_loop(0, NF, wait_body, 0)


@jax.jit
def pallas_adaLN_cond__mha_block_cached__geglu_ffn__prompt_kernel(
    A_x: jax.Array,
    A_k_cache: jax.Array,
    A_v_cache: jax.Array,
    A_wq: jax.Array,
    A_wo: jax.Array,
    B_x: jax.Array,
    B_w_gate: jax.Array,
    B_w_up: jax.Array,
    B_w_down: jax.Array,
    c: jax.Array,
    w_mod: jax.Array,
):
    del B_x
    x = A_x.reshape(SQ, D)
    k = A_k_cache.reshape(H, SK, DH)
    v = A_v_cache.reshape(H, SK, DH)
    any_spec = pl.BlockSpec(memory_space=pl.ANY)
    out = pl.pallas_call(
        _kernel,
        in_specs=[any_spec] * 10,
        out_specs=any_spec,
        out_shape=jax.ShapeDtypeStruct((SQ, D), A_x.dtype),
        scratch_shapes=[
            pltpu.VMEM((SQ, D), BF16),
            pltpu.VMEM((NSLOT, SK, DH), BF16),
            pltpu.VMEM((NSLOT, SK, DH), BF16),
            pltpu.VMEM((NSLOT, D, DH), BF16),
            pltpu.VMEM((NSLOT, DH, D), BF16),
            pltpu.VMEM((D, F), BF16),
            pltpu.VMEM((D, F), BF16),
            pltpu.VMEM((F, D), BF16),
            pltpu.VMEM((1, D), BF16),
            pltpu.VMEM((D, 6 * D), BF16),
            pltpu.VMEM((SQ, D), BF16),
            pltpu.VMEM((8, 6 * D), F32),
            pltpu.VMEM((SQ // 2, D), U32),
            pltpu.VMEM((SQ, D), F32),
            pltpu.VMEM((SQ // 2, D), U32),
            pltpu.VMEM((SQ, D), F32),
            [pltpu.VMEM((BF // 2 + PAD, FC), U32)] * NJ,
            [pltpu.VMEM((SQ // 2 + PAD, GW), U32)] * NG,
            [pltpu.VMEM((SQ + PAD, DH), F32)] * 2,
            [pltpu.VMEM((SQ + PAD, DH), F32)] * 2,
            [pltpu.VMEM((SQ + PAD, DH), F32)] * 2,
            pltpu.SemaphoreType.DMA((NSLOT, 4)),
            pltpu.SemaphoreType.DMA((6,)),
            pltpu.SemaphoreType.DMA((XC,)),
            pltpu.SemaphoreType.DMA((NF, NO)),
        ],
        compiler_params=pltpu.CompilerParams(
            vmem_limit_bytes=100 * 1024 * 1024,
        ),
    )(x, k, v, A_wq, A_wo, B_w_gate, B_w_up, B_w_down, c, w_mod)
    return out.reshape(A_x.shape)
```

```python
import numpy as np
import jax
import jax.numpy as jnp
import jax.experimental.pallas as pl
import jax.experimental.pallas.tpu as pltpu

H, DH, SQ, SK, D, F = 32, 128, 2048, 2048, 512, 1792
NG = 4
GW = SK // NG
BF = 512
NF = SQ // BF
FC = 896
NJ = F // FC
NSLOT = 4
XC = 8
XR = SQ // XC
NC = D // 128
NO = 4
OR = BF // NO
PAD = 8
QSC = float(DH ** -0.5 * np.log2(np.e))
F32, BF16, U32 = jnp.float32, jnp.bfloat16, jnp.uint32


def _packed(ref, *idx):
    return pltpu.bitcast(ref.bitcast(U32)[idx], BF16)


def _cols(v):
    return [v[:, c * 128:(c + 1) * 128] for c in range(v.shape[-1] // 128)]


def _adaln(xs, scale, shift, pins=None, never=None):
    m = jnp.sum((xs[0] + xs[1]) + (xs[2] + xs[3]), axis=-1, keepdims=True) * (1.0 / D)
    if pins is not None:
        m = jnp.where(never, pins[0], m)
    xc = [x - m for x in xs]
    v = jnp.sum((xc[0] * xc[0] + xc[1] * xc[1]) + (xc[2] * xc[2] + xc[3] * xc[3]),
                axis=-1, keepdims=True) * (1.0 / D)
    rs = jax.lax.rsqrt(v + 1e-5)
    if pins is not None:
        rs = jnp.where(never, pins[1], rs)
    return [a * rs * (1.0 + s) + t for a, s, t in zip(xc, _cols(scale), _cols(shift))]


def _kernel(x_hbm, k_hbm, v_hbm, wq_hbm, wo_hbm, wg_hbm, wu_hbm, wd_hbm, c_hbm, wm_hbm,
            o_hbm,
            x_v, k_v, v_v, wq_v, wo_v, wg_v, wu_v, wd_v, c_v, wm_v, o_v,
            mod_v, h_v, acc_v, h2_v, x1_v, fc_v, p_v, l_v, a_v, oa_v,
            sem_head, sem_misc, sem_x, sem_out):

    def slot_of(h):
        return h % NSLOT if isinstance(h, int) else h & (NSLOT - 1)

    def head_copies(h):
        g = min(h, H - 1) if isinstance(h, int) else jnp.minimum(h, H - 1)
        hc = pl.ds(pl.multiple_of(g * DH, DH), DH)
        s = slot_of(h)
        return (pltpu.make_async_copy(wq_hbm.at[:, hc], wq_v.at[s], sem_head.at[s, 0]),
                pltpu.make_async_copy(k_hbm.at[g], k_v.at[s], sem_head.at[s, 1]),
                pltpu.make_async_copy(v_hbm.at[g], v_v.at[s], sem_head.at[s, 2]),
                pltpu.make_async_copy(wo_hbm.at[hc, :], wo_v.at[s], sem_head.at[s, 3]))

    def start(h):
        for cp in head_copies(h):
            cp.start()

    def wait(h):
        for cp in head_copies(h):
            cp.wait()

    cp_c = pltpu.make_async_copy(c_hbm, c_v, sem_misc.at[0])
    cp_wma = pltpu.make_async_copy(wm_hbm.at[:, pl.ds(0, 2 * D)], wm_v.at[:, pl.ds(0, 2 * D)], sem_misc.at[1])
    cp_wmb = pltpu.make_async_copy(wm_hbm.at[:, pl.ds(2 * D, 4 * D)], wm_v.at[:, pl.ds(2 * D, 4 * D)], sem_misc.at[2])
    cp_ffn = [pltpu.make_async_copy(wg_hbm, wg_v, sem_misc.at[3]),
              pltpu.make_async_copy(wu_hbm, wu_v, sem_misc.at[4]),
              pltpu.make_async_copy(wd_hbm, wd_v, sem_misc.at[5])]
    cp_x = [pltpu.make_async_copy(x_hbm.at[pl.ds(j * XR, XR)], x_v.at[pl.ds(j * XR, XR)], sem_x.at[j])
            for j in range(XC)]

    cp_c.start()
    cp_wma.start()
    cp_x[0].start()
    cp_x[1].start()
    acc_v[...] = jnp.zeros((SQ, D), F32)

    cp_c.wait()
    c = c_v[...].astype(F32)
    sc = jnp.broadcast_to((c * jax.nn.sigmoid(c)).astype(BF16), (8, D))
    cp_wma.wait()
    cp_x[2].start()
    cp_x[3].start()
    mod_v[:, 0:2 * D] = jnp.dot(sc, wm_v[:, 0:2 * D], preferred_element_type=F32)

    def mod_row(k):
        return mod_v[0:1, k * D:(k + 1) * D]

    def ln1(j):
        r = pl.ds(j * XR, XR)
        xs = [x_v[r, pl.ds(c_ * 128, 128)].astype(F32) for c_ in range(NC)]
        for c_, hh in enumerate(_adaln(xs, mod_row(1), mod_row(0))):
            h_v[pl.ds(j * XR // 2, XR // 2), pl.ds(c_ * 128, 128)] = pltpu.bitcast(hh.astype(BF16), U32)

    cp_x[0].wait()
    ln1(0)
    cp_x[1].wait()
    for j in range(4, XC):
        cp_x[j].start()
    ln1(1)
    cp_x[2].wait()
    ln1(2)
    cp_x[3].wait()
    start(0)
    ln1(3)
    for j in range(4, XC):
        cp_x[j].wait()
    for j in range(4, XC):
        ln1(j)
    start(1)
    start(2)
    cp_wmb.start()

    def fence(ref, n, z):
        if z is not None:
            ref[pl.ds(pl.multiple_of(n + z, 8), 8), pl.ds(0, 128)] = jnp.zeros((8, 128), ref.dtype)

    def head(slot, z, post=None):
        q = jnp.dot(pltpu.bitcast(h_v[...], BF16), _packed(wq_v, slot), preferred_element_type=F32)
        q = (q * QSC).astype(BF16)
        st = {}

        def qk(g):
            kk = _packed(k_v, slot, pl.ds(g * GW // 2, GW // 2), slice(None))
            s = jax.lax.dot_general(q, kk, (((1,), (1,)), ((), ())), preferred_element_type=F32)
            mg = jnp.max(s, axis=-1, keepdims=True)
            if g == 0:
                m_new = mg
            else:
                m_new = jnp.maximum(st["m"], mg)
                alpha = jnp.exp2(st["m"] - m_new)
            p = jnp.exp2(s - m_new)
            lg = p[:, 0:128]
            for j in range(1, GW // 128):
                lg = lg + p[:, j * 128:(j + 1) * 128]
            if g > 0:
                lg = l_v[(g - 1) % 2][pl.ds(0, SQ), :] * alpha + lg
                a_v[g % 2][pl.ds(0, SQ), :] = jnp.broadcast_to(alpha, (SQ, DH))
                fence(a_v[g % 2], SQ, z)
            l_v[g % 2][pl.ds(0, SQ), :] = lg
            fence(l_v[g % 2], SQ, z)
            st["m"] = m_new
            p_v[g][pl.ds(0, SQ // 2), :] = pltpu.bitcast(p.astype(BF16), U32)
            fence(p_v[g], SQ // 2, z)

        def pv(g):
            vv = _packed(v_v, slot, pl.ds(g * GW // 2, GW // 2), slice(None))
            og = jnp.dot(pltpu.bitcast(p_v[g][pl.ds(0, SQ // 2), :], BF16), vv, preferred_element_type=F32)
            if g > 0:
                og = oa_v[(g - 1) % 2][pl.ds(0, SQ), :] * a_v[g % 2][pl.ds(0, SQ), :] + og
            if g + 1 < NG:
                oa_v[g % 2][pl.ds(0, SQ), :] = og
                fence(oa_v[g % 2], SQ, z)
            else:
                st["o"] = og

        qk(0); qk(1); pv(0); qk(2); pv(1); qk(3); pv(2); pv(3)
        l = jnp.sum(l_v[(NG - 1) % 2][pl.ds(0, SQ), :], axis=-1, keepdims=True)
        o = (st["o"] * (1.0 / l)).astype(BF16)
        new = acc_v[...] + jnp.dot(o, _packed(wo_v, slot), preferred_element_type=F32)
        acc_v[...] = new
        if post is not None:
            post(new)

    def head_body(h, carry):
        wait(h)
        head(slot_of(h), jax.lax.shift_right_logical(h, 16))
        start(h + 3)
        return carry | jax.lax.shift_right_logical(h, 16)
    z_out = jax.lax.fori_loop(0, H - 1, head_body, jnp.int32(0))

    def norm2(r0, attn, pins, never):
        r = pl.ds(r0, BF)
        r2 = pl.ds(r0 // 2 if isinstance(r0, int) else pl.multiple_of(r0 // 2, BF // 2), BF // 2)
        at = [acc_v[r, pl.ds(c_ * 128, 128)] for c_ in range(NC)] if attn is None else _cols(attn)
        xs = [x_v[r, pl.ds(c_ * 128, 128)].astype(F32) + g_ * a_
              for c_, (g_, a_) in enumerate(zip(_cols(mod_row(2)), at))]
        for c_, hh in enumerate(_adaln(xs, mod_row(4), mod_row(3), pins, never)):
            x1_v[r, pl.ds(c_ * 128, 128)] = xs[c_]
            h2_v[r2, pl.ds(c_ * 128, 128)] = pltpu.bitcast(hh.astype(BF16), U32)

    def first_norm2(attn):
        norm2(0, attn[0:BF], [attn[BF:2 * BF, 0:128], attn[2 * BF:3 * BF, 0:128]], z_out != 0)

    for cp in cp_ffn:
        cp.start()
    wait(H - 1)
    cp_wmb.wait()
    mod_v[:, 2 * D:6 * D] = jnp.dot(sc, wm_v[:, 2 * D:6 * D], preferred_element_type=F32)
    head(slot_of(H - 1), None, first_norm2)

    for cp in cp_ffn:
        cp.wait()

    def out_rows(i, t):
        return pl.ds(pl.multiple_of(i * BF + t * OR, OR), OR)

    def out_copy(i, t):
        return pltpu.make_async_copy(o_v.at[out_rows(i, t), :], o_hbm.at[out_rows(i, t), :], sem_out.at[i, t])

    def ffn_body(i, carry):
        r = pl.ds(pl.multiple_of(i * BF, BF), BF)
        z = jax.lax.shift_right_logical(i, 16)
        h2 = pltpu.bitcast(h2_v[pl.ds(pl.multiple_of(i * (BF // 2), BF // 2), BF // 2), :], BF16)
        for j in range(NJ):
            g = jnp.dot(h2, wg_v[:, pl.ds(j * FC, FC)], preferred_element_type=F32)
            u = jnp.dot(h2, wu_v[:, pl.ds(j * FC, FC)], preferred_element_type=F32)
            if j == 0:
                nxt = pl.multiple_of(jnp.minimum(i + 1, NF - 1) * BF, BF)
                norm2(nxt, None, [g[:, 0:128], g[:, FC - 128:FC]], z != 0)
            a = (jax.nn.gelu(g, approximate=True) * u).astype(BF16)
            fc_v[j][pl.ds(pl.multiple_of(z, BF // 2), BF // 2), :] = pltpu.bitcast(a, U32)
        aa = jnp.concatenate([pltpu.bitcast(fc_v[j][pl.ds(0, BF // 2), :], BF16) for j in range(NJ)], axis=1)
        y = jnp.dot(aa, wd_v[...], preferred_element_type=F32)
        res = (x1_v[r, :] + mod_row(5) * y).astype(o_v.dtype)
        for t in range(NO):
            o_v[out_rows(i, t), :] = res[t * OR:(t + 1) * OR]
            out_copy(i, t).start()
        return carry
    jax.lax.fori_loop(0, NF, ffn_body, 0)

    wait(H)
    wait(H + 1)

    def wait_body(i, carry):
        for t in range(NO):
            out_copy(i, t).wait()
        return carry
    jax.lax.fori_loop(0, NF, wait_body, 0)


@jax.jit
def pallas_adaLN_cond__mha_block_cached__geglu_ffn__prompt_kernel(
    A_x: jax.Array,
    A_k_cache: jax.Array,
    A_v_cache: jax.Array,
    A_wq: jax.Array,
    A_wo: jax.Array,
    B_x: jax.Array,
    B_w_gate: jax.Array,
    B_w_up: jax.Array,
    B_w_down: jax.Array,
    c: jax.Array,
    w_mod: jax.Array,
):
    del B_x
    x = A_x.reshape(SQ, D)
    k = A_k_cache.reshape(H, SK, DH)
    v = A_v_cache.reshape(H, SK, DH)
    any_spec = pl.BlockSpec(memory_space=pl.ANY)
    out = pl.pallas_call(
        _kernel,
        in_specs=[any_spec] * 10,
        out_specs=any_spec,
        out_shape=jax.ShapeDtypeStruct((SQ, D), A_x.dtype),
        scratch_shapes=[
            pltpu.VMEM((SQ, D), BF16),
            pltpu.VMEM((NSLOT, SK, DH), BF16),
            pltpu.VMEM((NSLOT, SK, DH), BF16),
            pltpu.VMEM((NSLOT, D, DH), BF16),
            pltpu.VMEM((NSLOT, DH, D), BF16),
            pltpu.VMEM((D, F), BF16),
            pltpu.VMEM((D, F), BF16),
            pltpu.VMEM((F, D), BF16),
            pltpu.VMEM((1, D), BF16),
            pltpu.VMEM((D, 6 * D), BF16),
            pltpu.VMEM((SQ, D), BF16),
            pltpu.VMEM((8, 6 * D), F32),
            pltpu.VMEM((SQ // 2, D), U32),
            pltpu.VMEM((SQ, D), F32),
            pltpu.VMEM((SQ // 2, D), U32),
            pltpu.VMEM((SQ, D), F32),
            [pltpu.VMEM((BF // 2 + PAD, FC), U32)] * NJ,
            [pltpu.VMEM((SQ // 2 + PAD, GW), U32)] * NG,
            [pltpu.VMEM((SQ + PAD, DH), F32)] * 2,
            [pltpu.VMEM((SQ + PAD, DH), F32)] * 2,
            [pltpu.VMEM((SQ + PAD, DH), F32)] * 2,
            pltpu.SemaphoreType.DMA((NSLOT, 4)),
            pltpu.SemaphoreType.DMA((6,)),
            pltpu.SemaphoreType.DMA((XC,)),
            pltpu.SemaphoreType.DMA((NF, NO)),
        ],
        compiler_params=pltpu.CompilerParams(
            vmem_limit_bytes=100 * 1024 * 1024,
        ),
    )(x, k, v, A_wq, A_wo, B_w_gate, B_w_up, B_w_down, c, w_mod)
    return out.reshape(A_x.shape)
```
